```python
import jax
import jax.numpy as jnp

def _softmax(x, axis=-1):
    return jax.nn.softmax(x, axis=axis)
def _gelu(x):
    return jax.nn.gelu(x, approximate=True)
def _silu(x):
    return jax.nn.silu(x)
def _sigmoid(x):
    return jax.nn.sigmoid(x)
def _layernorm(x, axis=-1, eps=1e-5):
    m = jnp.mean(x, axis=axis, keepdims=True)
    v = jnp.var(x, axis=axis, keepdims=True)
    return (x - m) / jnp.sqrt(v + eps)
def _scatter_add(tgt, idx, src, axis=0):
    return tgt.at[idx].add(src)
def _segment_sum(src, seg, n):
    return jax.ops.segment_sum(src, seg, n)
class _Rng:
    def __init__(self, key):
        self._k = key
    def _next(self):
        self._k, sub = jax.random.split(self._k)
        return sub
    def normal(self, shape):
        return jax.random.normal(self._next(), shape, dtype=jnp.bfloat16)
    def randint(self, lo, hi, shape):
        return jax.random.randint(self._next(), shape, lo, hi, dtype=jnp.int32)
    def uniform(self, shape, lo=0.0, hi=1.0):
        return jax.random.uniform(self._next(), shape, jnp.bfloat16, lo, hi)
    def permutation(self, n):
        return jax.random.permutation(self._next(), n)


kernel_name = 'standalone__modern_conv_block_slak__vision'

def setup_inputs():
    _rng = _Rng(jax.random.key(int.from_bytes(__import__("os").urandom(4), "little")))
    _w = (lambda a: (lambda t: t.astype(jnp.bfloat16) if jnp.issubdtype(t.dtype, jnp.floating) else t)(jnp.asarray(a)))
    H = W = 384
    C = 384
    K = 1
    return {
        "x": _w((lambda *s: _rng.normal(s) * 0.05)(1, H, W, C)),
        "dw": _w((lambda *s: _rng.normal(s) * 0.05)(K, K, C)),
        "w1": _w((lambda *s: _rng.normal(s) * 0.05)(C, 4 * C)),
        "w2": _w((lambda *s: _rng.normal(s) * 0.05)(4 * C, C)),
        "grn_g": _w((lambda *s: _rng.normal(s) * 0.05)(4 * C)),
        "grn_b": _w((lambda *s: _rng.normal(s) * 0.05)(4 * C)),
    }

def reference(x, dw, w1, w2, grn_g, grn_b):
    B, H, W, C = x.shape
    K = dw.shape[0]
    pad = K // 2
    xp = jnp.pad(x, ((0,0),(pad,pad),(pad,pad),(0,0)))
    out = jnp.zeros_like(x)
    for i in range(K):
        for j in range(K):
            out = out + xp[:, i:i+H, j:j+W, :] * dw[i, j][None, None, None, :]
    h = _layernorm(out, axis=-1)
    h = _gelu(h @ w1)
    gx = jnp.sqrt((h * h).sum(axis=(1, 2), keepdims=True) + 1e-6)
    nx = gx / (gx.mean(axis=-1, keepdims=True) + 1e-6)
    h = grn_g[None, None, None, :] * (h * nx) + grn_b[None, None, None, :] + h
    return x + h @ w2
```

```python
import functools
import jax
import jax.numpy as jnp
from jax.experimental import pallas as pl
from jax.experimental.pallas import tpu as pltpu

C0 = 0.7978845608028654
C1 = C0 * 0.044715
ALPHA = C1 ** (1.0 / 3.0)
BETA = C0 / ALPHA
F32 = jnp.float32
BF16 = jnp.bfloat16


def _kernel(x_ref, dw_ref, w1_ref, w2_ref, g_ref, b_ref, o_ref, h_hbm,
            h_buf, ssq_ref, w2s_ref, bias_ref, wsem, rsem, *, tm, tn, nt, phases):
    p = pl.program_id(0)
    i = pl.program_id(1)
    slot = i % 2
    c = x_ref.shape[1]
    c4 = w1_ref.shape[1]

    def wcopy(s, t):
        return pltpu.make_async_copy(h_buf.at[s], h_hbm.at[pl.ds(t * tm, tm)], wsem.at[s])

    def rcopy(s, t):
        return pltpu.make_async_copy(h_hbm.at[pl.ds(t * tm, tm)], h_buf.at[s], rsem.at[s])

    @pl.when(p == 0)
    def _phase0():
        @pl.when(i == 0)
        def _():
            ssq_ref[...] = jnp.zeros(ssq_ref.shape, F32)

        @pl.when(i >= 2)
        def _():
            wcopy(slot, i - 2).wait()

        y = x_ref[...].astype(F32) * dw_ref[...].astype(F32)
        m = jnp.mean(y, axis=-1, keepdims=True)
        yc = y - m
        v = jnp.mean(yc * yc, axis=-1, keepdims=True)
        r = jax.lax.rsqrt(v + 1e-5) * ALPHA
        xn = (yc * r).astype(BF16)
        for j in range(c4 // tn):
            sl = slice(j * tn, (j + 1) * tn)
            z = jnp.dot(xn, w1_ref[:, sl], preferred_element_type=F32)
            t = jnp.tanh(z * (z * z + BETA))
            g = z * (t + 1.0)
            ssq_ref[:, sl] += jnp.sum((g * g).reshape(tm // 8, 8, tn), axis=0)
            h_buf[slot, :, sl] = g.astype(BF16)
        wcopy(slot, i).start()

    @pl.when(p == 1)
    def _phase1():
        @pl.when(i == 0)
        def _():
            wcopy((nt - 2) % 2, nt - 2).wait()
            wcopy((nt - 1) % 2, nt - 1).wait()
            rcopy(0, 0).start()
            inv = 1.0 / (2.0 * ALPHA)
            ss = jnp.sum(ssq_ref[...], axis=0, keepdims=True) * (inv * inv)
            gx = jnp.sqrt(ss + 1e-6)
            nx = gx / (jnp.mean(gx, axis=-1, keepdims=True) + 1e-6)
            s = (g_ref[...].astype(F32) * nx + 1.0) * inv
            st = jnp.transpose(jnp.broadcast_to(s, (128, c4)))
            for jc in range(c // 128):
                cs = slice(jc * 128, (jc + 1) * 128)
                w2s_ref[:, cs] = (w2_ref[:, cs].astype(F32) * st).astype(BF16)
            bb = jnp.broadcast_to(b_ref[...], (8, c4))
            bias_ref[...] = jnp.dot(bb, w2_ref[...], preferred_element_type=F32)

        @pl.when(i + 1 < nt)
        def _():
            rcopy(1 - slot, i + 1).start()

        rcopy(slot, i).wait()
        acc = jnp.dot(h_buf[slot], w2s_ref[...], preferred_element_type=F32)
        o_ref[...] = (acc + x_ref[...].astype(F32) + bias_ref[0:1, :]).astype(o_ref.dtype)


@jax.jit
def pallas_standalone__modern_conv_block_slak__vision_kernel(x, dw, w1, w2, grn_g, grn_b):
    tm, tn, vmem_mb = 2048, 512, 100
    B, H, W, C = x.shape
    n = B * H * W
    c4 = w1.shape[1]
    nt = n // tm
    x2 = x.reshape(n, C)
    kern = functools.partial(_kernel, tm=tm, tn=tn, nt=nt, phases=2)
    const = lambda p, i: (0, 0)
    out, _ = pl.pallas_call(
        kern,
        grid=(2, nt),
        in_specs=[
            pl.BlockSpec((tm, C), lambda p, i: (i, 0)),
            pl.BlockSpec((1, C), const),
            pl.BlockSpec((C, c4), const),
            pl.BlockSpec((c4, C), const),
            pl.BlockSpec((1, c4), const),
            pl.BlockSpec((1, c4), const),
        ],
        out_specs=[
            pl.BlockSpec((tm, C), lambda p, i: (i * p, 0)),
            pl.BlockSpec(memory_space=pl.ANY),
        ],
        out_shape=[jax.ShapeDtypeStruct((n, C), x.dtype),
                   jax.ShapeDtypeStruct((n, c4), BF16)],
        scratch_shapes=[
            pltpu.VMEM((2, tm, c4), BF16),
            pltpu.VMEM((8, c4), F32),
            pltpu.VMEM((c4, C), BF16),
            pltpu.VMEM((8, C), F32),
            pltpu.SemaphoreType.DMA((2,)),
            pltpu.SemaphoreType.DMA((2,)),
        ],
        compiler_params=pltpu.CompilerParams(
            dimension_semantics=("arbitrary", "arbitrary"),
            vmem_limit_bytes=vmem_mb * 1024 * 1024),
    )(x2, dw.reshape(1, C), w1, w2, grn_g.reshape(1, c4), grn_b.reshape(1, c4))
    return out.reshape(B, H, W, C)
```

```python
import functools
import jax
import jax.numpy as jnp
from jax.experimental import pallas as pl
from jax.experimental.pallas import tpu as pltpu

C0 = 0.7978845608028654
C1 = C0 * 0.044715
ALPHA = C1 ** (1.0 / 3.0)
BETA = C0 / ALPHA
F32 = jnp.float32
BF16 = jnp.bfloat16


def _kernel(x_ref, xh_ref, dw_ref, w1_ref, w2_ref, g_ref, b_ref, o_ref, h_hbm,
            ring, xn0_ref, ssq_ref, w2s_ref, bias_ref, wsem, rsem,
            *, tm, ts, tn, ts2, nt, nb, ln_first):
    p = pl.program_id(0)
    i = pl.program_id(1)
    ns = nt - nb
    c = x_ref.shape[1]
    c4 = w1_ref.shape[1]
    nr = tm // ts

    def wcopy(s, t):
        return pltpu.make_async_copy(ring.at[s], h_hbm.at[pl.ds(t * tm, tm)], wsem.at[s])

    def rcopy(s, t):
        return pltpu.make_async_copy(h_hbm.at[pl.ds(t * tm, tm)], ring.at[s], rsem.at[s])

    def layernorm(xv):
        y = xv.astype(F32) * dw_ref[...].astype(F32)
        m = jnp.mean(y, axis=-1, keepdims=True)
        yc = y - m
        v = jnp.mean(yc * yc, axis=-1, keepdims=True)
        r = jax.lax.rsqrt(v + 1e-5) * ALPHA
        return (yc * r).astype(BF16)

    @pl.when(p == 0)
    def _phase0():
        slot = i % nb

        @pl.when(i == 0)
        def _():
            ssq_ref[...] = jnp.zeros(ssq_ref.shape, F32)
            xn0_ref[...] = layernorm(x_ref[0:ts, :])

        @pl.when(i >= nb)
        def _():
            wcopy(slot, i - nb).wait()

        xn = xn0_ref[...]
        for k in range(nr):
            def next_ln():
                if k + 1 < nr:
                    return layernorm(x_ref[(k + 1) * ts:(k + 2) * ts, :])
                return layernorm(xh_ref[...])
            if ln_first:
                xn_next = next_ln()
            for j in range(c4 // tn):
                sl = slice(j * tn, (j + 1) * tn)
                z = jnp.dot(xn, w1_ref[:, sl], preferred_element_type=F32)
                t = jnp.tanh(z * (z * z + BETA))
                g = z * (t + 1.0)
                ssq_ref[:, sl] += jnp.sum((g * g).reshape(ts // 8, 8, tn), axis=0)
                ring[slot, k * ts:(k + 1) * ts, sl] = g.astype(BF16)
            if not ln_first:
                xn_next = next_ln()
            xn = xn_next
        xn0_ref[...] = xn

        @pl.when(i < ns)
        def _():
            wcopy(slot, i).start(priority=1)

    @pl.when(p == 1)
    def _phase1():
        slot = (ns + i) % nb

        @pl.when(i == 0)
        def _():
            inv = 1.0 / (2.0 * ALPHA)
            ss = jnp.sum(ssq_ref[...], axis=0, keepdims=True) * (inv * inv)
            gx = jnp.sqrt(ss + 1e-6)
            nx = gx / (jnp.mean(gx, axis=-1, keepdims=True) + 1e-6)
            s = (g_ref[...].astype(F32) * nx + 1.0) * inv
            st = jnp.transpose(jnp.broadcast_to(s, (128, c4)))
            for jc in range(c // 128):
                cs = slice(jc * 128, (jc + 1) * 128)
                w2s_ref[:, cs] = (w2_ref[:, cs].astype(F32) * st).astype(BF16)
            bb = jnp.broadcast_to(b_ref[...], (8, c4))
            bias_ref[...] = jnp.dot(bb, w2_ref[...], preferred_element_type=F32)

        @pl.when(i >= nb)
        def _():
            rcopy(slot, i - nb).wait()

        for k in range(tm // ts2):
            rs = slice(k * ts2, (k + 1) * ts2)
            acc = jnp.dot(ring[slot, rs, :], w2s_ref[...], preferred_element_type=F32)
            o_ref[rs, :] = (acc + x_ref[rs, :].astype(F32) + bias_ref[0:1, :]).astype(o_ref.dtype)

        @pl.when(i < ns)
        def _():
            rcopy(slot, i).start(priority=1)


@jax.jit
def pallas_standalone__modern_conv_block_slak__vision_kernel(x, dw, w1, w2, grn_g, grn_b):
    tm, ts, tn, nb, vmem_mb, ln_first = 4096, 128, 1536, 6, 120, True
    ts2 = tm
    B, H, W, C = x.shape
    n = B * H * W
    c4 = w1.shape[1]
    nt = n // tm
    ns = nt - nb
    nr = tm // ts
    x2 = x.reshape(n, C)
    kern = functools.partial(_kernel, tm=tm, ts=ts, tn=tn, ts2=ts2, nt=nt, nb=nb, ln_first=ln_first)
    const = lambda p, i: (0, 0)
    rot = lambda i: jnp.where(i + ns >= nt, i + ns - nt, i + ns)
    tile = lambda p, i: jnp.where(p == 0, i, rot(i))
    one = pl.Buffered(1)
    out, _ = pl.pallas_call(
        kern,
        grid=(2, nt),
        in_specs=[
            pl.BlockSpec((tm, C), lambda p, i: (tile(p, i), 0)),
            pl.BlockSpec((ts, C), lambda p, i: (jnp.where(p == 0, jnp.minimum(i + 1, nt - 1), nt - 1) * nr, 0)),
            pl.BlockSpec((1, C), const, pipeline_mode=one),
            pl.BlockSpec((C, c4), const, pipeline_mode=one),
            pl.BlockSpec((c4, C), const, pipeline_mode=one),
            pl.BlockSpec((1, c4), const, pipeline_mode=one),
            pl.BlockSpec((1, c4), const, pipeline_mode=one),
        ],
        out_specs=[
            pl.BlockSpec((tm, C), lambda p, i: (jnp.where(p == 0, ns, rot(i)), 0)),
            pl.BlockSpec(memory_space=pl.ANY),
        ],
        out_shape=[jax.ShapeDtypeStruct((n, C), x.dtype),
                   jax.ShapeDtypeStruct((ns * tm, c4), BF16)],
        scratch_shapes=[
            pltpu.VMEM((nb, tm, c4), BF16),
            pltpu.VMEM((ts, C), BF16),
            pltpu.VMEM((8, c4), F32),
            pltpu.VMEM((c4, C), BF16),
            pltpu.VMEM((8, C), F32),
            pltpu.SemaphoreType.DMA((nb,)),
            pltpu.SemaphoreType.DMA((nb,)),
        ],
        compiler_params=pltpu.CompilerParams(
            dimension_semantics=("arbitrary", "arbitrary"),
            disable_bounds_checks=True,
            vmem_limit_bytes=vmem_mb * 1024 * 1024),
    )(x2, x2, dw.reshape(1, C), w1, w2, grn_g.reshape(1, c4), grn_b.reshape(1, c4))
    return out.reshape(B, H, W, C)
```

```python
import functools
import jax
import jax.numpy as jnp
from jax import lax
from jax.experimental import pallas as pl
from jax.experimental.pallas import tpu as pltpu

C0 = 0.7978845608028654
C1 = C0 * 0.044715
ALPHA = C1 ** (1.0 / 3.0)
BETA = C0 / ALPHA
F32 = jnp.float32
BF16 = jnp.bfloat16
U32 = jnp.uint32
NX = 3
L = 128


def _mm(a, b):
    return jnp.dot(a, b, preferred_element_type=F32)


def _ld(ref_u32_view, *idx):
    return pltpu.bitcast(ref_u32_view[idx], BF16)


def _kernel(x_hbm, dw_hbm, w1_hbm, w2_hbm, g_hbm, b_hbm, o_hbm, h_hbm,
            xbuf, obuf, ring, ssq_ref, dw_ref, w1_ref, w2_ref, g_ref, b_ref,
            w2c_ref, w23_ref, w1c_ref, lhs0_ref, bias_ref,
            xsem, osem, wsem, rsem, psem,
            *, tm, ts, nt, nb, m2):
    ns = nt - nb
    c4 = w1_hbm.shape[1]
    nk = c4 // L
    nh = nk // 2
    nr = tm // ts

    ring_u = ring.bitcast(U32)
    w1_u = w1_ref.bitcast(U32)
    w2c_u = w2c_ref.bitcast(U32)
    w23_u = w23_ref.bitcast(U32)
    w1c_u = w1c_ref.bitcast(U32)

    def rows(t):
        return pl.ds(pl.multiple_of(t * tm, 128), tm)

    def xtile(s):
        return jnp.where(s < nt, s, jnp.where(s - nb >= nt, s - nb - nt, s - nb))

    def xcopy(slot, s):
        return pltpu.make_async_copy(x_hbm.at[rows(xtile(s))], xbuf.at[slot], xsem.at[slot])

    def ocopy(slot, t):
        return pltpu.make_async_copy(obuf.at[slot], o_hbm.at[rows(t)], osem.at[slot])

    def wcopy(s, t):
        return pltpu.make_async_copy(ring.at[s], h_hbm.at[t], wsem.at[s])

    def rcopy(s, t):
        return pltpu.make_async_copy(h_hbm.at[t], ring.at[s], rsem.at[s])

    def layernorm(xv):
        y = xv.astype(F32) * dw_ref[...].astype(F32)
        mu = jnp.mean(y, axis=-1, keepdims=True)
        yc = y - mu
        var = jnp.mean(yc * yc, axis=-1, keepdims=True)
        xn = yc * (lax.rsqrt(var + 1e-5) * ALPHA)
        m = ts // 2
        a11, a12, a3a = xn[:m, 0:L], xn[:m, L:2 * L], xn[:m, 2 * L:3 * L]
        a21, a22, a3b = xn[m:, 0:L], xn[m:, L:2 * L], xn[m:, 2 * L:3 * L]
        return tuple(v.astype(BF16) for v in
                     (a11 + a22, a21 + a22, a11, a22, a11 + a12, a21 - a11, a12 - a22, a3a, a3b))

    def lhs_store(t):
        for q, v in enumerate(t):
            lhs0_ref[q] = v

    def act(z, slot, j, r0, nrows):
        t = jnp.tanh(z * (z * z + BETA))
        g = z * (t + 1.0)
        ssq_ref[:, j * L:(j + 1) * L] += jnp.sum((g * g).reshape(nrows // 8, 8, L), axis=0)
        ring[slot, j, r0:r0 + nrows, :] = g.astype(BF16)

    def inc(v, n):
        return jnp.where(v + 1 >= n, 0, v + 1)

    cp_dw = pltpu.make_async_copy(dw_hbm, dw_ref, psem.at[0])
    cp_x0 = pltpu.make_async_copy(x_hbm.at[pl.ds(0, ts)], xbuf.at[0, pl.ds(0, ts)], psem.at[1])
    cp_w1 = [pltpu.make_async_copy(w1_hbm.at[:, pl.ds(j * L, L)], w1_ref.at[j], psem.at[2])
             for j in range(nk)]
    cp_x0r = pltpu.make_async_copy(x_hbm.at[pl.ds(ts, tm - ts)], xbuf.at[0, pl.ds(ts, tm - ts)],
                                   psem.at[3])
    cp_w2 = pltpu.make_async_copy(w2_hbm, w2_ref, psem.at[4])
    cp_g = pltpu.make_async_copy(g_hbm, g_ref, psem.at[5])
    cp_b = pltpu.make_async_copy(b_hbm, b_ref, psem.at[6])
    cp_dw.start()
    cp_x0.start()
    for cp in cp_w1:
        cp.start()
    cp_x0r.start()
    xcopy(1, 1).start(priority=1)
    cp_w2.start(priority=1)
    cp_g.start(priority=1)
    cp_b.start(priority=1)
    ssq_ref[...] = jnp.zeros(ssq_ref.shape, F32)
    cp_dw.wait()
    cp_x0.wait()
    lhs_store(layernorm(xbuf[0, 0:ts, :]))
    pltpu.make_async_copy(w1_ref, w1_ref, psem.at[2]).wait()
    for cc in range(nh):
        b11 = w1_ref[cc, 0:L, :].astype(F32)
        b21 = w1_ref[cc, L:2 * L, :].astype(F32)
        b12 = w1_ref[nh + cc, 0:L, :].astype(F32)
        b22 = w1_ref[nh + cc, L:2 * L, :].astype(F32)
        for q, v in enumerate([b11 + b22, b11, b12 - b22, b21 - b11, b22, b11 + b12, b21 + b22]):
            w1c_ref[q, cc] = v.astype(BF16)
    cp_x0r.wait()

    def phase0(i, carry):
        xs, slot = carry
        xs1 = inc(xs, NX)
        xs2 = inc(xs1, NX)
        xcopy(xs2, i + 2).start()
        xcopy(xs1, i + 1).wait()

        @pl.when(i >= nb)
        def _():
            wcopy(slot, i - nb).wait()

        m = ts // 2
        lhs = tuple(lhs0_ref[q] for q in range(9))
        for k in range(nr):
            if k + 1 < nr:
                lhs_next = layernorm(xbuf[xs, (k + 1) * ts:(k + 2) * ts, :])
            else:
                lhs_next = layernorm(xbuf[xs1, 0:ts, :])
            a3 = jnp.concatenate([lhs[7], lhs[8]], axis=0)
            for cc in range(nh):
                p1, p2, p3, p4, p5, p6, p7 = [_mm(lhs[q], _ld(w1c_u, q, cc)) for q in range(7)]
                s1 = _mm(a3, _ld(w1_u, cc, slice(L, 3 * L // 2)))
                s2 = _mm(a3, _ld(w1_u, nh + cc, slice(L, 3 * L // 2)))
                act(p1 + p4 - p5 + p7 + s1[:m], slot, cc, k * ts, m)
                act(p3 + p5 + s2[:m], slot, nh + cc, k * ts, m)
                act(p2 + p4 + s1[m:], slot, cc, k * ts + m, m)
                act(p1 - p2 + p3 + p6 + s2[m:], slot, nh + cc, k * ts + m, m)
            lhs = lhs_next
        lhs_store(lhs)

        @pl.when(i < ns)
        def _():
            wcopy(slot, i).start(priority=1)

        return xs1, inc(slot, nb)

    xs, slot = lax.fori_loop(0, nt, phase0, (jnp.int32(0), jnp.int32(0)))

    cp_w2.wait()
    cp_g.wait()
    cp_b.wait()
    inv = 1.0 / (2.0 * ALPHA)
    ss = jnp.sum(ssq_ref[...], axis=0, keepdims=True) * (inv * inv)
    gx = jnp.sqrt(ss + 1e-6)
    nx = gx / (jnp.mean(gx, axis=-1, keepdims=True) + 1e-6)
    s = (g_ref[...].astype(F32) * nx + 1.0) * inv
    st = jnp.transpose(jnp.broadcast_to(s, (L, c4)))
    kh = c4 // 2
    wc = [w2_ref[:, jc * L:(jc + 1) * L].astype(F32) * st for jc in range(3)]
    b11, b21 = wc[0][:kh], wc[0][kh:]
    b12, b22 = wc[1][:kh], wc[1][kh:]
    for q, v in enumerate([b11 + b22, b11, b12 - b22, b21 - b11, b22, b11 + b12, b21 + b22]):
        w2c_ref[q] = v.astype(BF16)
    w23_ref[...] = wc[2].astype(BF16)
    bias_ref[...] = _mm(jnp.broadcast_to(b_ref[...], (8, c4)), w2_ref[...])

    def phase1(j, carry):
        xs, slot, osl = carry
        sidx = nt + j
        xs1 = inc(xs, NX)
        xs2 = inc(xs1, NX)

        @pl.when(j + 2 < nt)
        def _():
            xcopy(xs2, sidx + 2).start()

        @pl.when(j + 1 < nt)
        def _():
            xcopy(xs1, sidx + 1).wait()

        @pl.when(j >= nb)
        def _():
            rcopy(slot, j - nb).wait()

        @pl.when(j >= 2)
        def _():
            ocopy(osl, 0).wait()

        def A(rs, k0, k1):
            rh = slice(rs.start // 2, rs.stop // 2)
            return jnp.concatenate([_ld(ring_u, slot, kt, rh) for kt in range(k0, k1)], axis=1)

        def fin(v, rs, cs):
            obuf[osl, rs, cs] = (v + xbuf[xs, rs, cs].astype(F32) + bias_ref[0:1, cs]).astype(BF16)

        add = lambda u, v: (u.astype(F32) + v.astype(F32)).astype(BF16)
        sub = lambda u, v: (u.astype(F32) - v.astype(F32)).astype(BF16)
        for k in range(tm // (2 * m2)):
            r1 = slice(2 * k * m2, (2 * k + 1) * m2)
            r2 = slice((2 * k + 1) * m2, (2 * k + 2) * m2)
            r12 = slice(2 * k * m2, (2 * k + 2) * m2)
            p1 = _mm(add(A(r1, 0, nh), A(r2, nh, nk)), _ld(w2c_u, 0))
            p2 = _mm(add(A(r2, 0, nh), A(r2, nh, nk)), _ld(w2c_u, 1))
            p3 = _mm(A(r1, 0, nh), _ld(w2c_u, 2))
            p4 = _mm(A(r2, nh, nk), _ld(w2c_u, 3))
            p5 = _mm(add(A(r1, 0, nh), A(r1, nh, nk)), _ld(w2c_u, 4))
            p6 = _mm(sub(A(r2, 0, nh), A(r1, 0, nh)), _ld(w2c_u, 5))
            p7 = _mm(sub(A(r1, nh, nk), A(r2, nh, nk)), _ld(w2c_u, 6))
            c3 = _mm(A(r12, 0, nk), pltpu.bitcast(w23_u[...], BF16))
            fin(p1 + p4 - p5 + p7, r1, slice(0, L))
            fin(p3 + p5, r1, slice(L, 2 * L))
            fin(p2 + p4, r2, slice(0, L))
            fin(p1 - p2 + p3 + p6, r2, slice(L, 2 * L))
            fin(c3, r12, slice(2 * L, 3 * L))
        ocopy(osl, xtile(sidx)).start()

        @pl.when(j < ns)
        def _():
            rcopy(slot, j).start(priority=1)

        return xs1, inc(slot, nb), 1 - osl

    lax.fori_loop(0, nt, phase1, (xs, slot, jnp.int32(0)))
    ocopy(0, 0).wait()
    ocopy(1, 0).wait()


@jax.jit
def pallas_standalone__modern_conv_block_slak__vision_kernel(x, dw, w1, w2, grn_g, grn_b):
    tm, ts, nb, m2 = 3072, 64, 10, 256
    B, H, W, C = x.shape
    n = B * H * W
    c4 = w1.shape[1]
    nk = c4 // L
    nt = n // tm
    ns = nt - nb
    assert n % tm == 0 and C == 3 * L and dw.shape[:2] == (1, 1)
    kern = functools.partial(_kernel, tm=tm, ts=ts, nt=nt, nb=nb, m2=m2)
    any_spec = pl.BlockSpec(memory_space=pl.ANY)
    out, _ = pl.pallas_call(
        kern,
        in_specs=[any_spec] * 6,
        out_specs=[any_spec, any_spec],
        out_shape=[jax.ShapeDtypeStruct((n, C), x.dtype),
                   jax.ShapeDtypeStruct((ns, nk, tm, L), BF16)],
        scratch_shapes=[
            pltpu.VMEM((NX, tm, C), BF16),
            pltpu.VMEM((2, tm, C), BF16),
            pltpu.VMEM((nb, nk, tm, L), BF16),
            pltpu.VMEM((8, c4), F32),
            pltpu.VMEM((1, C), BF16),
            pltpu.VMEM((nk, C, L), BF16),
            pltpu.VMEM((c4, C), BF16),
            pltpu.VMEM((1, c4), BF16),
            pltpu.VMEM((1, c4), BF16),
            pltpu.VMEM((7, c4 // 2, L), BF16),
            pltpu.VMEM((c4, L), BF16),
            pltpu.VMEM((7, nk // 2, L, L), BF16),
            pltpu.VMEM((9, ts // 2, L), BF16),
            pltpu.VMEM((8, C), F32),
            pltpu.SemaphoreType.DMA((NX,)),
            pltpu.SemaphoreType.DMA((2,)),
            pltpu.SemaphoreType.DMA((nb,)),
            pltpu.SemaphoreType.DMA((nb,)),
            pltpu.SemaphoreType.DMA((7,)),
        ],
        compiler_params=pltpu.CompilerParams(
            disable_bounds_checks=True,
            vmem_limit_bytes=127 * 1024 * 1024),
    )(x.reshape(n, C), dw.reshape(1, C), w1, w2, grn_g.reshape(1, c4), grn_b.reshape(1, c4))
    return out.reshape(B, H, W, C)
```

```python
import functools
import jax
import jax.numpy as jnp
from jax import lax
from jax.experimental import pallas as pl
from jax.experimental.pallas import tpu as pltpu

C0 = 0.7978845608028654
C1 = C0 * 0.044715
ALPHA = C1 ** (1.0 / 3.0)
BETA = C0 / ALPHA
F32 = jnp.float32
BF16 = jnp.bfloat16
U32 = jnp.uint32
NX = 3
L = 128

_U = [[[0, 1, -1], [0, 0, -1]], [[0, 1, -1], [0, 0, 0]], [[1, 0, 0], [1, 0, 0]], [[0, 0, 0], [1, 0, 1]],
      [[0, 1, -1], [0, 1, -1]], [[1, 0, 0], [1, 1, 0]], [[0, 0, 1], [0, 0, 1]], [[1, 0, 1], [0, 0, 0]],
      [[0, 1, 0], [0, 0, 0]], [[0, 0, 0], [0, 0, 1]], [[0, 0, 0], [0, 1, 0]], [[0, 0, 0], [1, 1, 0]],
      [[1, 1, 0], [1, 1, 0]], [[1, 0, 0], [0, 0, -1]], [[1, 0, 0], [0, 0, 0]]]
_V = [[[0, 0, 0], [0, 0, 1], [0, -1, 0]], [[0, 0, 0], [0, 0, 0], [0, 1, 0]], [[1, 0, -1], [-1, 0, 0], [0, 0, 0]],
      [[0, 0, 1], [0, 0, 0], [0, 0, 0]], [[0, 0, 0], [0, 0, 1], [0, 0, 0]], [[0, 1, 0], [1, 0, 0], [0, 0, 0]],
      [[0, 0, 0], [0, 0, 1], [-1, 0, 1]], [[0, 0, 0], [0, 0, 0], [1, 0, 0]], [[0, 0, 0], [1, 1, 0], [0, 1, 0]],
      [[0, 0, 1], [0, 0, 0], [0, -1, -1]], [[0, 1, 0], [0, -1, -1], [0, 0, 0]], [[0, 1, 0], [0, 0, 0], [0, 0, 0]],
      [[0, 0, 0], [1, 0, 0], [0, 0, 0]], [[0, 0, 1], [0, 0, 0], [-1, 0, 0]], [[1, 1, 0], [0, 0, 0], [-1, 0, 0]]]
_W = [[[0, 0, 1], [0, 1, -1]], [[0, -1, 1], [0, 1, -1]], [[0, 0, 0], [1, 0, 0]], [[0, 0, 0], [1, 0, 1]],
      [[0, 0, 0], [0, -1, 1]], [[-1, 1, 0], [1, 0, 0]], [[0, 0, 1], [0, 0, 0]], [[1, 0, 1], [0, 0, 0]],
      [[0, 1, 0], [0, 0, 0]], [[0, 0, 1], [0, 0, -1]], [[0, 0, 0], [0, -1, 0]], [[1, -1, 0], [-1, 1, 0]],
      [[1, -1, 0], [0, 0, 0]], [[0, 0, 1], [1, 0, 0]], [[1, 0, 0], [-1, 0, 0]]]
NP = 15


def _plan(rows):
    rows = [dict(r) for r in rows]
    steps = []
    nv = 1000
    while True:
        cnt = {}
        for r in rows:
            ks = sorted(r)
            for i in range(len(ks)):
                for j in range(i + 1, len(ks)):
                    key = (ks[i], ks[j], r[ks[i]] * r[ks[j]])
                    cnt[key] = cnt.get(key, 0) + 1
        if not cnt:
            break
        key, c = max(cnt.items(), key=lambda kv: kv[1])
        if c < 2:
            break
        a, b, s = key
        nv += 1
        steps.append((nv, a, b, s))
        for r in rows:
            if a in r and b in r and r[a] * r[b] == s:
                sg = r[a]
                del r[a], r[b]
                r[nv] = sg
    return steps, rows


def _signed_sum(items):
    pos = [t for s, t in items if s > 0]
    neg = [t for s, t in items if s < 0]
    if pos:
        v = pos[0]()
        for t in pos[1:]:
            v = v + t()
        for t in neg:
            v = v - t()
        return v
    v = neg[0]()
    for t in neg[1:]:
        v = v + t()
    return -v


def _eval_plan(plan, vals):
    steps, rows = plan
    vals = dict(vals)
    for nv, a, b, s in steps:
        vals[nv] = vals[a] + vals[b] if s > 0 else vals[a] - vals[b]
    return [_signed_sum([(sg, (lambda k=k: vals[k])) for k, sg in r.items()]) for r in rows]


_A_ROWS = [{i * 3 + j: _U[r][i][j] for i in range(2) for j in range(3) if _U[r][i][j]} for r in range(NP)]
_B_ROWS = [{j * 3 + l: _V[r][j][l] for j in range(3) for l in range(3) if _V[r][j][l]} for r in range(NP)]
_C_ROWS = [{r: _W[r][i][l] for r in range(NP) if _W[r][i][l]} for i in range(2) for l in range(3)]
_A_PLAN = _plan(_A_ROWS)
_B_PLAN = ([], _B_ROWS)
_C_PLAN = _plan(_C_ROWS)


def _mm(a, b):
    return jnp.dot(a, b, preferred_element_type=F32)


def _ld(ref_u32_view, *idx):
    return pltpu.bitcast(ref_u32_view[idx], BF16)


def _kernel(x_hbm, dw_hbm, w1_hbm, w2_hbm, g_hbm, b_hbm, o_hbm, h_hbm,
            xbuf, obuf, ring, ssq_ref, dw_ref, g_ref, b_ref,
            w1c_ref, w2c_ref, lhs0_ref, bias_ref, zero_ref,
            xsem, osem, wsem, rsem, psem,
            *, tm, ts, nq, nt, nb, m2, o0, o1):
    ns = nt - nb
    c = x_hbm.shape[1]
    c4 = w1_hbm.shape[1]
    nk = c4 // L
    n3 = nk // 3
    nr = tm // ts
    tq = tm // nq

    ring_u = ring.bitcast(U32)
    w1c_u = w1c_ref.bitcast(U32)
    w2c_u = w2c_ref.bitcast(U32)
    order0 = [int(ch, 16) for ch in o0]
    order1 = [int(ch, 16) for ch in o1]

    def rows(t, n=tm, off=0):
        return pl.ds(pl.multiple_of(t * tm + off, 128), n)

    def xtile(s):
        return jnp.where(s < nt, s, jnp.where(s - nb >= nt, s - nb - nt, s - nb))

    def xcopy(slot, s):
        return pltpu.make_async_copy(x_hbm.at[rows(xtile(s))], xbuf.at[slot], xsem.at[slot])

    def ocopy(slot, t, q):
        return pltpu.make_async_copy(obuf.at[slot, pl.ds(q * tq, tq)], o_hbm.at[rows(t, tq, q * tq)], osem.at[slot])

    def owait(slot):
        pltpu.make_async_copy(obuf.at[slot], obuf.at[slot], osem.at[slot]).wait()

    def wcopy(s, t):
        return pltpu.make_async_copy(ring.at[pl.ds(s * nq, nq)], h_hbm.at[pl.ds(t * nq, nq)], wsem.at[s])

    def rcopy(s, t, q):
        return pltpu.make_async_copy(h_hbm.at[t * nq + q], ring.at[s * nq + q], rsem.at[s * nq + q])

    def layernorm(xv):
        y = xv.astype(F32) * dw_ref[...].astype(F32)
        mu = jnp.mean(y, axis=-1, keepdims=True)
        yc = y - mu
        var = jnp.mean(yc * yc, axis=-1, keepdims=True)
        xn = yc * (lax.rsqrt(var + 1e-5) * ALPHA)
        m = ts // 2
        blocks = {i * 3 + j: xn[i * m:(i + 1) * m, j * L:(j + 1) * L] for i in range(2) for j in range(3)}
        return tuple(v.astype(BF16) for v in _eval_plan(_A_PLAN, blocks))

    def lhs_store(t):
        for q, v in enumerate(t):
            lhs0_ref[q] = v

    def act(z, slot, j, r0, nrows):
        t = jnp.tanh(z * (z * z + BETA))
        g = z * (t + 1.0)
        ssq_ref[:, j * L:(j + 1) * L] += jnp.sum((g * g).reshape(nrows // 8, 8, L), axis=0)
        ring[slot * nq + r0 // tq, j, r0 % tq:r0 % tq + nrows, :] = g.astype(BF16)

    def inc(v, n):
        return jnp.where(v + 1 >= n, 0, v + 1)

    w1_stage = ring.at[nb * nq - 1]
    w2_stage = obuf.at[0, pl.ds(0, c4)]
    cp_dw = pltpu.make_async_copy(dw_hbm, dw_ref, psem.at[0])
    cp_x0 = pltpu.make_async_copy(x_hbm.at[pl.ds(0, ts)], xbuf.at[0, pl.ds(0, ts)], psem.at[1])
    cp_w1 = [pltpu.make_async_copy(w1_hbm.at[:, pl.ds(j * L, L)], w1_stage.at[j, pl.ds(0, c)], psem.at[2])
             for j in range(nk)]
    cp_x0r = pltpu.make_async_copy(x_hbm.at[pl.ds(ts, tm - ts)], xbuf.at[0, pl.ds(ts, tm - ts)], psem.at[3])
    cp_w2 = pltpu.make_async_copy(w2_hbm, w2_stage, psem.at[4])
    cp_g = pltpu.make_async_copy(g_hbm, g_ref, psem.at[5])
    cp_b = pltpu.make_async_copy(b_hbm, b_ref, psem.at[6])
    cp_dw.start()
    cp_x0.start()
    for cp in cp_w1:
        cp.start()
    cp_x0r.start()
    xcopy(1, 1).start(priority=1)
    cp_w2.start(priority=1)
    cp_g.start(priority=1)
    cp_b.start(priority=1)
    ssq_ref[...] = jnp.zeros(ssq_ref.shape, F32)
    for q in range(16):
        zero_ref[q] = 0
    cp_dw.wait()
    cp_x0.wait()
    lhs_store(layernorm(xbuf[0, 0:ts, :]))
    w1_all = w1_stage.at[:, pl.ds(0, c)]
    pltpu.make_async_copy(w1_all, w1_all, psem.at[2]).wait()
    for cc in range(n3):
        blocks = {j * 3 + l: ring[nb * nq - 1, l * n3 + cc, j * L:(j + 1) * L, :].astype(F32)
                  for j in range(3) for l in range(3)}
        for q, v in enumerate(_eval_plan(_B_PLAN, blocks)):
            w1c_ref[q, cc] = v.astype(BF16)
    cp_x0r.wait()

    def phase0(i, carry):
        xs, slot = carry
        xs1 = inc(xs, NX)
        xs2 = inc(xs1, NX)
        xcopy(xs2, i + 2).start()
        xcopy(xs1, i + 1).wait()

        @pl.when(i >= nb)
        def _():
            wcopy(slot, i - nb).wait()

        m = ts // 2
        lhs = tuple(lhs0_ref[q] for q in range(NP))
        for k in range(nr):
            if k + 1 < nr:
                lhs_next = layernorm(xbuf[xs, (k + 1) * ts:(k + 2) * ts, :])
            else:
                lhs_next = layernorm(xbuf[xs1, 0:ts, :])
            for cc in range(n3):
                P = {}
                for r in order0:
                    P[r] = _mm(lhs[r], _ld(w1c_u, r, cc))
                for o, v in enumerate(_eval_plan(_C_PLAN, P)):
                    act(v, slot, (o % 3) * n3 + cc, k * ts + (o // 3) * m, m)
            lhs = lhs_next
        lhs_store(lhs)

        @pl.when(i < ns)
        def _():
            wcopy(slot, i).start(priority=1)

        return xs1, inc(slot, nb)

    xs, slot = lax.fori_loop(0, nt, phase0, (jnp.int32(0), jnp.int32(0)))

    cp_w2.wait()
    cp_g.wait()
    cp_b.wait()
    inv = 1.0 / (2.0 * ALPHA)
    ss = jnp.sum(ssq_ref[...], axis=0, keepdims=True) * (inv * inv)
    gx = jnp.sqrt(ss + 1e-6)
    nx = gx / (jnp.mean(gx, axis=-1, keepdims=True) + 1e-6)
    s = (g_ref[...].astype(F32) * nx + 1.0) * inv
    st = jnp.transpose(jnp.broadcast_to(s, (L, c4)))
    k3 = c4 // 3
    wc = [obuf[0, 0:c4, l * L:(l + 1) * L].astype(F32) * st for l in range(3)]
    blocks = {j * 3 + l: wc[l][j * k3:(j + 1) * k3] for j in range(3) for l in range(3)}
    for q, v in enumerate(_eval_plan(_B_PLAN, blocks)):
        w2c_ref[q] = v.astype(BF16)
    bias_ref[...] = _mm(jnp.broadcast_to(b_ref[...], (8, c4)), obuf[0, 0:c4, :])

    def phase1(j, carry):
        xs, slot, osl = carry
        sidx = nt + j
        xs1 = inc(xs, NX)
        xs2 = inc(xs1, NX)

        @pl.when(j + 2 < nt)
        def _():
            xcopy(xs2, sidx + 2).start()

        @pl.when(j + 1 < nt)
        def _():
            xcopy(xs1, sidx + 1).wait()

        @pl.when(j >= 2)
        def _():
            owait(osl)

        tile = xtile(sidx)
        base = [slot * nq + zero_ref[r] for r in range(NP)]

        def A(r, row0, jk):
            q, rr = row0 // tq, row0 % tq
            rh = slice(rr // 2, (rr + m2) // 2)
            return jnp.concatenate([_ld(ring_u, base[r] + q, kt, rh) for kt in range(jk * n3, (jk + 1) * n3)], axis=1)

        per_q = tq // (2 * m2)
        for k in range(tm // (2 * m2)):
            q = k // per_q
            if k % per_q == 0:
                @pl.when(j >= nb)
                def _():
                    rcopy(slot, j - nb, q).wait()
            r0 = (2 * k * m2, (2 * k + 1) * m2)
            P = {}
            for r in order1:
                terms = [(_U[r][i_][j_], (lambda i_=i_, j_=j_: A(r, r0[i_], j_))) for i_ in range(2) for j_ in range(3) if _U[r][i_][j_]]
                if len(terms) == 1:
                    assert terms[0][0] == 1
                    lhs_ = terms[0][1]()
                else:
                    lhs_ = _signed_sum([(sg, (lambda t=t: t().astype(F32))) for sg, t in terms]).astype(BF16)
                P[r] = _mm(lhs_, _ld(w2c_u, r))
            for o, v in enumerate(_eval_plan(_C_PLAN, P)):
                rs = slice(r0[o // 3], r0[o // 3] + m2)
                cs = slice((o % 3) * L, (o % 3 + 1) * L)
                obuf[osl, rs, cs] = (v + xbuf[xs, rs, cs].astype(F32) + bias_ref[0:1, cs]).astype(BF16)
            if (k + 1) % per_q == 0:
                ocopy(osl, tile, q).start()

                @pl.when(j < ns)
                def _():
                    rcopy(slot, j, q).start(priority=1)

        return xs1, inc(slot, nb), 1 - osl

    lax.fori_loop(0, nt, phase1, (xs, slot, jnp.int32(0)))
    owait(0)
    owait(1)


@jax.jit
def pallas_standalone__modern_conv_block_slak__vision_kernel(x, dw, w1, w2, grn_g, grn_b):
    tm, ts, nq, nb, vmem_mb, m2 = 3072, 64, 3, 12, 128, 256
    o0, o1 = '82b015ce97a364d', '0123456789abcde'
    B, H, W, C = x.shape
    n = B * H * W
    c4 = w1.shape[1]
    nk = c4 // L
    nt = n // tm
    assert n % tm == 0 and C == 3 * L and c4 == 12 * L and dw.shape[:2] == (1, 1)
    ns = nt - nb
    tq = tm // nq
    kern = functools.partial(_kernel, tm=tm, ts=ts, nq=nq, nt=nt, nb=nb, m2=m2, o0=o0, o1=o1)
    any_spec = pl.BlockSpec(memory_space=pl.ANY)
    out, _ = pl.pallas_call(
        kern,
        in_specs=[any_spec] * 6,
        out_specs=[any_spec, any_spec],
        out_shape=[jax.ShapeDtypeStruct((n, C), x.dtype),
                   jax.ShapeDtypeStruct((ns * nq, nk, tq, L), BF16)],
        scratch_shapes=[
            pltpu.VMEM((NX, tm, C), BF16),
            pltpu.VMEM((2, tm, C), BF16),
            pltpu.VMEM((nb * nq, nk, tq, L), BF16),
            pltpu.VMEM((8, c4), F32),
            pltpu.VMEM((1, C), BF16),
            pltpu.VMEM((1, c4), BF16),
            pltpu.VMEM((1, c4), BF16),
            pltpu.VMEM((NP, nk // 3, L, L), BF16),
            pltpu.VMEM((NP, c4 // 3, L), BF16),
            pltpu.VMEM((NP, ts // 2, L), BF16),
            pltpu.VMEM((8, C), F32),
            pltpu.SMEM((16,), jnp.int32),
            pltpu.SemaphoreType.DMA((NX,)),
            pltpu.SemaphoreType.DMA((2,)),
            pltpu.SemaphoreType.DMA((nb,)),
            pltpu.SemaphoreType.DMA((nb * nq,)),
            pltpu.SemaphoreType.DMA((7,)),
        ],
        compiler_params=pltpu.CompilerParams(
            disable_bounds_checks=True,
            vmem_limit_bytes=vmem_mb * 1024 * 1024),
    )(x.reshape(n, C), dw.reshape(1, C), w1, w2, grn_g.reshape(1, c4), grn_b.reshape(1, c4))
    return out.reshape(B, H, W, C)
```

```python
import functools
import jax
import jax.numpy as jnp
from jax import lax
from jax.experimental import pallas as pl
from jax.experimental.pallas import tpu as pltpu

C0 = 0.7978845608028654
C1 = C0 * 0.044715
ALPHA = C1 ** (1.0 / 3.0)
BETA = C0 / ALPHA
F32 = jnp.float32
BF16 = jnp.bfloat16
U32 = jnp.uint32
NX = 3
L = 128

_U = [[[0, 1, -1], [0, 0, -1]], [[0, 1, -1], [0, 0, 0]], [[1, 0, 0], [1, 0, 0]], [[0, 0, 0], [1, 0, 1]],
      [[0, 1, -1], [0, 1, -1]], [[1, 0, 0], [1, 1, 0]], [[0, 0, 1], [0, 0, 1]], [[1, 0, 1], [0, 0, 0]],
      [[0, 1, 0], [0, 0, 0]], [[0, 0, 0], [0, 0, 1]], [[0, 0, 0], [0, 1, 0]], [[0, 0, 0], [1, 1, 0]],
      [[1, 1, 0], [1, 1, 0]], [[1, 0, 0], [0, 0, -1]], [[1, 0, 0], [0, 0, 0]]]
_V = [[[0, 0, 0], [0, 0, 1], [0, -1, 0]], [[0, 0, 0], [0, 0, 0], [0, 1, 0]], [[1, 0, -1], [-1, 0, 0], [0, 0, 0]],
      [[0, 0, 1], [0, 0, 0], [0, 0, 0]], [[0, 0, 0], [0, 0, 1], [0, 0, 0]], [[0, 1, 0], [1, 0, 0], [0, 0, 0]],
      [[0, 0, 0], [0, 0, 1], [-1, 0, 1]], [[0, 0, 0], [0, 0, 0], [1, 0, 0]], [[0, 0, 0], [1, 1, 0], [0, 1, 0]],
      [[0, 0, 1], [0, 0, 0], [0, -1, -1]], [[0, 1, 0], [0, -1, -1], [0, 0, 0]], [[0, 1, 0], [0, 0, 0], [0, 0, 0]],
      [[0, 0, 0], [1, 0, 0], [0, 0, 0]], [[0, 0, 1], [0, 0, 0], [-1, 0, 0]], [[1, 1, 0], [0, 0, 0], [-1, 0, 0]]]
_W = [[[0, 0, 1], [0, 1, -1]], [[0, -1, 1], [0, 1, -1]], [[0, 0, 0], [1, 0, 0]], [[0, 0, 0], [1, 0, 1]],
      [[0, 0, 0], [0, -1, 1]], [[-1, 1, 0], [1, 0, 0]], [[0, 0, 1], [0, 0, 0]], [[1, 0, 1], [0, 0, 0]],
      [[0, 1, 0], [0, 0, 0]], [[0, 0, 1], [0, 0, -1]], [[0, 0, 0], [0, -1, 0]], [[1, -1, 0], [-1, 1, 0]],
      [[1, -1, 0], [0, 0, 0]], [[0, 0, 1], [1, 0, 0]], [[1, 0, 0], [-1, 0, 0]]]
NP = 15
assert all(
    sum(_U[r][i][j] * _V[r][p][l] * _W[r][a][b] for r in range(NP)) == int(j == p and i == a and l == b)
    for i in range(2) for j in range(3) for p in range(3) for l in range(3) for a in range(2) for b in range(3))


def _plan(rows):
    rows = [dict(r) for r in rows]
    steps = []
    nv = 1000
    while True:
        cnt = {}
        for r in rows:
            ks = sorted(r)
            for i in range(len(ks)):
                for j in range(i + 1, len(ks)):
                    key = (ks[i], ks[j], r[ks[i]] * r[ks[j]])
                    cnt[key] = cnt.get(key, 0) + 1
        if not cnt:
            break
        key, c = max(cnt.items(), key=lambda kv: kv[1])
        if c < 2:
            break
        a, b, s = key
        nv += 1
        steps.append((nv, a, b, s))
        for r in rows:
            if a in r and b in r and r[a] * r[b] == s:
                sg = r[a]
                del r[a], r[b]
                r[nv] = sg
    return steps, rows


def _signed_sum(items):
    pos = [t for s, t in items if s > 0]
    neg = [t for s, t in items if s < 0]
    if pos:
        v = pos[0]()
        for t in pos[1:]:
            v = v + t()
        for t in neg:
            v = v - t()
        return v
    v = neg[0]()
    for t in neg[1:]:
        v = v + t()
    return -v


def _eval_plan(plan, vals):
    steps, rows = plan
    vals = dict(vals)
    for nv, a, b, s in steps:
        vals[nv] = vals[a] + vals[b] if s > 0 else vals[a] - vals[b]
    return [_signed_sum([(sg, (lambda k=k: vals[k])) for k, sg in r.items()]) for r in rows]


_A_ROWS = [{i * 3 + j: _U[r][i][j] for i in range(2) for j in range(3) if _U[r][i][j]} for r in range(NP)]
_B_ROWS = [{j * 3 + l: _V[r][j][l] for j in range(3) for l in range(3) if _V[r][j][l]} for r in range(NP)]
_C_ROWS = [{r: _W[r][i][l] for r in range(NP) if _W[r][i][l]} for i in range(2) for l in range(3)]
_A_PLAN = _plan(_A_ROWS)
_B_PLAN = ([], _B_ROWS)
_C_PLAN = _plan(_C_ROWS)


def _mm(a, b):
    return jnp.dot(a, b, preferred_element_type=F32)


def _ld(ref_u32_view, *idx):
    return pltpu.bitcast(ref_u32_view[idx], BF16)


def _kernel(x_hbm, dw_hbm, w1_hbm, w2_hbm, g_hbm, b_hbm, o_hbm, h_hbm,
            xbuf, hbuf, ring, ssq_ref, dw_ref, g_ref, b_ref,
            wc_ref, lhs0_ref, bias_ref, zero_ref,
            xsem, hsem, osem, wsem, rsem, psem,
            *, tm, ts, nq, nt, nb, m2, o0, o1):
    ns = nt - nb
    c = x_hbm.shape[1]
    c4 = w1_hbm.shape[1]
    nk = c4 // L
    n3 = nk // 3
    nr = tm // ts
    tq = tm // nq
    m = ts // 2

    ring_u = ring.bitcast(U32)
    wc_u = wc_ref.bitcast(U32)
    order0 = [int(ch, 16) for ch in o0]
    order1 = [int(ch, 16) for ch in o1]

    def rows(t, n=tm, off=0):
        return pl.ds(pl.multiple_of(t * tm + off, 128), n)

    def rot(j):
        if isinstance(j, int):
            return nt - 1 - j if j < nb else j - nb
        return jnp.where(j < nb, nt - 1 - j, j - nb)

    def xcopy(slot, t):
        return pltpu.make_async_copy(x_hbm.at[rows(t)], xbuf.at[slot], xsem.at[slot])

    def hcopy(slot, t):
        return pltpu.make_async_copy(x_hbm.at[rows(t, ts)], hbuf.at[slot], hsem.at[slot])

    def ocopy(slot, t, q):
        return pltpu.make_async_copy(xbuf.at[slot, pl.ds(q * tq, tq)], o_hbm.at[rows(t, tq, q * tq)],
                                     osem.at[slot])

    def owait(slot, t):
        for q in range(nq):
            ocopy(slot, t, q).wait()

    def wcopy(s, t):
        return pltpu.make_async_copy(ring.at[pl.ds(s * nq, nq)], h_hbm.at[pl.ds(t * nq, nq)], wsem.at[s])

    def rcopy(s, t, q):
        return pltpu.make_async_copy(h_hbm.at[t * nq + q], ring.at[s * nq + q], rsem.at[s * nq + q])

    def layernorm(xv):
        y = xv.astype(F32) * dw_ref[...].astype(F32)
        mu = jnp.sum(y, axis=-1, keepdims=True) * (1.0 / c)
        yc = y - mu
        var = jnp.mean(yc * yc, axis=-1, keepdims=True)
        xn = yc * (lax.rsqrt(var + 1e-5) * ALPHA)
        blocks = {i * 3 + j: xn[i * m:(i + 1) * m, j * L:(j + 1) * L] for i in range(2) for j in range(3)}
        return tuple(v.astype(BF16) for v in _eval_plan(_A_PLAN, blocks))

    def lhs_store(t):
        for q, v in enumerate(t):
            lhs0_ref[q] = v

    def act(z, slot, j, r0):
        t = jnp.tanh(z * (z * z + BETA))
        g = z * (t + 1.0)
        ssq_ref[:, j * L:(j + 1) * L] += jnp.sum((g * g).reshape(m // 8, 8, L), axis=0)
        rr = (j % n3) * tq + r0 % tq
        ring[slot * nq + r0 // tq, j // n3, rr:rr + m, :] = g.astype(BF16)

    def inc(v, n):
        return jnp.where(v + 1 >= n, 0, v + 1)

    def dec(v, n):
        return jnp.where(v == 0, n - 1, v - 1)

    last = nb * nq - 1
    cp_dw = pltpu.make_async_copy(dw_hbm, dw_ref, psem.at[0])
    cp_w1 = [pltpu.make_async_copy(w1_hbm.at[:, pl.ds(j * L, L)],
                                   ring.at[last, j // n3, pl.ds((j % n3) * tq, c)], psem.at[1])
             for j in range(nk)]
    cp_w2 = pltpu.make_async_copy(w2_hbm, xbuf.at[2, pl.ds(0, c4)], psem.at[2])
    cp_g = pltpu.make_async_copy(g_hbm, g_ref, psem.at[3])
    cp_b = pltpu.make_async_copy(b_hbm, b_ref, psem.at[4])
    cp_dw.start()
    hcopy(0, 0).start()
    for cp in cp_w1:
        cp.start()
    hcopy(1, 1).start()
    xcopy(0, 0).start(priority=1)
    cp_w2.start(priority=1)
    cp_g.start(priority=1)
    cp_b.start(priority=1)
    ssq_ref[...] = jnp.zeros(ssq_ref.shape, F32)
    for q in range(NP):
        zero_ref[q] = 0
    cp_dw.wait()
    hcopy(0, 0).wait()
    lhs_store(layernorm(hbuf[0]))
    for cp in cp_w1:
        cp.wait()
    for cc in range(n3):
        blocks = {j * 3 + l: ring[last, l, cc * tq + j * L:cc * tq + (j + 1) * L, :].astype(F32)
                  for j in range(3) for l in range(3)}
        for q, v in enumerate(_eval_plan(_B_PLAN, blocks)):
            wc_ref[q, cc * L:(cc + 1) * L, :] = v.astype(BF16)

    def phase0(i, carry):
        xs, slot = carry
        xs1 = 1 - xs
        xcopy(xs, i).wait()
        hcopy(xs1, jnp.minimum(i + 1, nt - 1)).wait()

        @pl.when(i + 1 < nt)
        def _():
            xcopy(xs1, i + 1).start()
            hcopy(xs, jnp.minimum(i + 2, nt - 1)).start()

        @pl.when(i >= nb)
        def _():
            wcopy(slot, i - nb).wait()

        lhs = tuple(lhs0_ref[q] for q in range(NP))
        for k in range(nr):
            if k + 1 < nr:
                lhs_next = layernorm(xbuf[xs, (k + 1) * ts:(k + 2) * ts, :])
            else:
                lhs_next = layernorm(hbuf[xs1])
            for cc in range(n3):
                P = {}
                for r in order0:
                    P[r] = _mm(lhs[r], _ld(wc_u, r, slice(cc * L // 2, (cc + 1) * L // 2)))
                for o, v in enumerate(_eval_plan(_C_PLAN, P)):
                    act(v, slot, (o % 3) * n3 + cc, k * ts + (o // 3) * m)
            lhs = lhs_next
        lhs_store(lhs)

        @pl.when(i < ns)
        def _():
            wcopy(slot, i).start(priority=1)

        return xs1, inc(slot, nb)

    lax.fori_loop(0, nt, phase0, (jnp.int32(0), jnp.int32(0)))

    cp_w2.wait()
    cp_g.wait()
    cp_b.wait()
    inv = 1.0 / (2.0 * ALPHA)
    ss = jnp.sum(ssq_ref[...], axis=0, keepdims=True) * (inv * inv)
    gx = jnp.sqrt(ss + 1e-6)
    nx = gx / (jnp.mean(gx, axis=-1, keepdims=True) + 1e-6)
    s = (g_ref[...].reshape(1, c4).astype(F32) * nx + 1.0) * inv
    k3 = c4 // 3
    for rb in range(k3 // L):
        blocks = {}
        for j in range(3):
            r0 = j * k3 + rb * L
            st = jnp.transpose(jnp.broadcast_to(s[:, r0:r0 + L], (L, L)))
            for l in range(3):
                blocks[j * 3 + l] = xbuf[2, r0:r0 + L, l * L:(l + 1) * L].astype(F32) * st
        for q, v in enumerate(_eval_plan(_B_PLAN, blocks)):
            wc_ref[q, rb * L:(rb + 1) * L, :] = v.astype(BF16)
    bias_ref[...] = _mm(jnp.broadcast_to(b_ref[...].reshape(1, c4), (8, c4)), xbuf[2, 0:c4, :])

    def phase1(j, carry):
        xs, slot = carry
        xs1 = dec(xs, NX)

        @pl.when(j >= 2)
        def _():
            owait(xs1, rot(j - 2))

        @pl.when(jnp.logical_and(j >= 1, j + 1 < nt))
        def _():
            xcopy(xs1, rot(j + 1)).start()

        @pl.when(j >= 2)
        def _():
            xcopy(xs, rot(j)).wait()

        tile = rot(j)
        base = [slot * nq + zero_ref[r] for r in range(NP)]

        def A(r, row0, jk):
            q = row0 // tq
            cols = []
            for kt in range(n3):
                rr = kt * tq + row0 % tq
                cols.append(_ld(ring_u, base[r] + q, jk, slice(rr // 2, (rr + m2) // 2)))
            return jnp.concatenate(cols, axis=1)

        per_q = tq // (2 * m2)
        for k in range(tm // (2 * m2)):
            q = k // per_q
            if k % per_q == 0:
                @pl.when(j >= nb)
                def _():
                    rcopy(slot, j - nb, q).wait()
            r0 = (2 * k * m2, (2 * k + 1) * m2)
            P = {}
            for r in order1:
                terms = [(_U[r][i_][j_], (lambda i_=i_, j_=j_: A(r, r0[i_], j_)))
                         for i_ in range(2) for j_ in range(3) if _U[r][i_][j_]]
                if len(terms) == 1:
                    assert terms[0][0] == 1
                    lhs = terms[0][1]()
                else:
                    lhs = _signed_sum([(sg, (lambda t=t: t().astype(F32))) for sg, t in terms]).astype(BF16)
                P[r] = _mm(lhs, _ld(wc_u, r))
            for o, v in enumerate(_eval_plan(_C_PLAN, P)):
                rs = slice(r0[o // 3], r0[o // 3] + m2)
                cs = slice((o % 3) * L, (o % 3 + 1) * L)
                xbuf[xs, rs, cs] = (v + xbuf[xs, rs, cs].astype(F32) + bias_ref[0:1, cs]).astype(BF16)
            if (k + 1) % per_q == 0:
                ocopy(xs, tile, q).start()

                @pl.when(j < ns)
                def _():
                    rcopy(slot, j, q).start(priority=1)

        return xs1, dec(slot, nb)

    lax.fori_loop(0, nt, phase1, (jnp.int32(1), jnp.int32((nt - 1) % nb)))
    owait((1 - (nt - 2)) % NX, rot(nt - 2))
    owait((1 - (nt - 1)) % NX, rot(nt - 1))


@jax.jit
def pallas_standalone__modern_conv_block_slak__vision_kernel(x, dw, w1, w2, grn_g, grn_b):
    tm, ts, nq, nb, m2 = 3072, 64, 3, 13, 128
    o0, o1 = '01b825ce97a64d3', '0123456789abcde'
    B, H, W, C = x.shape
    n = B * H * W
    c4 = w1.shape[1]
    nk = c4 // L
    nt = n // tm
    ns = nt - nb
    tq = tm // nq
    assert n % tm == 0 and nt % 2 == 0 and C == 3 * L and c4 == 12 * L and dw.shape[:2] == (1, 1)
    kern = functools.partial(_kernel, tm=tm, ts=ts, nq=nq, nt=nt, nb=nb, m2=m2, o0=o0, o1=o1)
    any_spec = pl.BlockSpec(memory_space=pl.ANY)
    out, _ = pl.pallas_call(
        kern,
        in_specs=[any_spec] * 6,
        out_specs=[any_spec, any_spec],
        out_shape=[jax.ShapeDtypeStruct((n, C), x.dtype),
                   jax.ShapeDtypeStruct((ns * nq, 3, nk // 3 * tq, L), BF16)],
        scratch_shapes=[
            pltpu.VMEM((NX, tm, C), BF16),
            pltpu.VMEM((2, ts, C), BF16),
            pltpu.VMEM((nb * nq, 3, nk // 3 * tq, L), BF16),
            pltpu.VMEM((8, c4), F32),
            pltpu.VMEM((1, C), BF16),
            pltpu.VMEM((c4,), BF16),
            pltpu.VMEM((c4,), BF16),
            pltpu.VMEM((NP, c4 // 3, L), BF16),
            pltpu.VMEM((NP, ts // 2, L), BF16),
            pltpu.VMEM((8, C), F32),
            pltpu.SMEM((NP,), jnp.int32),
            pltpu.SemaphoreType.DMA((NX,)),
            pltpu.SemaphoreType.DMA((2,)),
            pltpu.SemaphoreType.DMA((NX,)),
            pltpu.SemaphoreType.DMA((nb,)),
            pltpu.SemaphoreType.DMA((nb * nq,)),
            pltpu.SemaphoreType.DMA((5,)),
        ],
        compiler_params=pltpu.CompilerParams(
            disable_bounds_checks=True,
            vmem_limit_bytes=128 * 1024 * 1024),
    )(x.reshape(n, C), dw.reshape(1, C), w1, w2, grn_g, grn_b)
    return out.reshape(B, H, W, C)
```

```python
import functools
import jax
import jax.numpy as jnp
from jax import lax
from jax.experimental import pallas as pl
from jax.experimental.pallas import tpu as pltpu

C0 = 0.7978845608028654
C1 = C0 * 0.044715
ALPHA = C1 ** (1.0 / 3.0)
BETA = C0 / ALPHA
F32 = jnp.float32
BF16 = jnp.bfloat16
U32 = jnp.uint32
NX = 3
L = 128

_U = [[[0, 1, -1], [0, 0, -1]], [[0, 1, -1], [0, 0, 0]], [[1, 0, 0], [1, 0, 0]], [[0, 0, 0], [1, 0, 1]],
      [[0, 1, -1], [0, 1, -1]], [[1, 0, 0], [1, 1, 0]], [[0, 0, 1], [0, 0, 1]], [[1, 0, 1], [0, 0, 0]],
      [[0, 1, 0], [0, 0, 0]], [[0, 0, 0], [0, 0, 1]], [[0, 0, 0], [0, 1, 0]], [[0, 0, 0], [1, 1, 0]],
      [[1, 1, 0], [1, 1, 0]], [[1, 0, 0], [0, 0, -1]], [[1, 0, 0], [0, 0, 0]]]
_V = [[[0, 0, 0], [0, 0, 1], [0, -1, 0]], [[0, 0, 0], [0, 0, 0], [0, 1, 0]], [[1, 0, -1], [-1, 0, 0], [0, 0, 0]],
      [[0, 0, 1], [0, 0, 0], [0, 0, 0]], [[0, 0, 0], [0, 0, 1], [0, 0, 0]], [[0, 1, 0], [1, 0, 0], [0, 0, 0]],
      [[0, 0, 0], [0, 0, 1], [-1, 0, 1]], [[0, 0, 0], [0, 0, 0], [1, 0, 0]], [[0, 0, 0], [1, 1, 0], [0, 1, 0]],
      [[0, 0, 1], [0, 0, 0], [0, -1, -1]], [[0, 1, 0], [0, -1, -1], [0, 0, 0]], [[0, 1, 0], [0, 0, 0], [0, 0, 0]],
      [[0, 0, 0], [1, 0, 0], [0, 0, 0]], [[0, 0, 1], [0, 0, 0], [-1, 0, 0]], [[1, 1, 0], [0, 0, 0], [-1, 0, 0]]]
_W = [[[0, 0, 1], [0, 1, -1]], [[0, -1, 1], [0, 1, -1]], [[0, 0, 0], [1, 0, 0]], [[0, 0, 0], [1, 0, 1]],
      [[0, 0, 0], [0, -1, 1]], [[-1, 1, 0], [1, 0, 0]], [[0, 0, 1], [0, 0, 0]], [[1, 0, 1], [0, 0, 0]],
      [[0, 1, 0], [0, 0, 0]], [[0, 0, 1], [0, 0, -1]], [[0, 0, 0], [0, -1, 0]], [[1, -1, 0], [-1, 1, 0]],
      [[1, -1, 0], [0, 0, 0]], [[0, 0, 1], [1, 0, 0]], [[1, 0, 0], [-1, 0, 0]]]
NP = 15
assert all(
    sum(_U[r][i][j] * _V[r][p][l] * _W[r][a][b] for r in range(NP)) == int(j == p and i == a and l == b)
    for i in range(2) for j in range(3) for p in range(3) for l in range(3) for a in range(2) for b in range(3))


def _plan(rows):
    rows = [dict(r) for r in rows]
    steps = []
    nv = 1000
    while True:
        cnt = {}
        for r in rows:
            ks = sorted(r)
            for i in range(len(ks)):
                for j in range(i + 1, len(ks)):
                    key = (ks[i], ks[j], r[ks[i]] * r[ks[j]])
                    cnt[key] = cnt.get(key, 0) + 1
        if not cnt:
            break
        key, c = max(cnt.items(), key=lambda kv: kv[1])
        if c < 2:
            break
        a, b, s = key
        nv += 1
        steps.append((nv, a, b, s))
        for r in rows:
            if a in r and b in r and r[a] * r[b] == s:
                sg = r[a]
                del r[a], r[b]
                r[nv] = sg
    return steps, rows


def _signed_sum(items):
    pos = [t for s, t in items if s > 0]
    neg = [t for s, t in items if s < 0]
    if pos:
        v = pos[0]()
        for t in pos[1:]:
            v = v + t()
        for t in neg:
            v = v - t()
        return v
    v = neg[0]()
    for t in neg[1:]:
        v = v + t()
    return -v


def _eval_plan(plan, vals):
    steps, rows = plan
    vals = dict(vals)
    for nv, a, b, s in steps:
        vals[nv] = vals[a] + vals[b] if s > 0 else vals[a] - vals[b]
    return [_signed_sum([(sg, (lambda k=k: vals[k])) for k, sg in r.items()]) for r in rows]


_A_ROWS = [{i * 3 + j: _U[r][i][j] for i in range(2) for j in range(3) if _U[r][i][j]} for r in range(NP)]
_B_ROWS = [{j * 3 + l: _V[r][j][l] for j in range(3) for l in range(3) if _V[r][j][l]} for r in range(NP)]
_C_ROWS = [{r: _W[r][i][l] for r in range(NP) if _W[r][i][l]} for i in range(2) for l in range(3)]
_A_PLAN = _plan(_A_ROWS)
_B_PLAN = ([], _B_ROWS)
_C_PLAN = _plan(_C_ROWS)


def _mm(a, b):
    return jnp.dot(a, b, preferred_element_type=F32)


def _pack(v):
    return pltpu.bitcast(v.astype(BF16), U32)


def _unpack(v):
    return pltpu.bitcast(v, BF16)


def _kernel(x_hbm, dw_hbm, w1_hbm, w2_hbm, g_hbm, b_hbm, o_hbm, h_hbm,
            xbuf, hbuf, ring, ssq_ref, dw_ref, g_ref, b_ref,
            wc_ref, lhs0_ref, bias_ref, zero_ref,
            xsem, hsem, osem, wsem, rsem, psem,
            *, tm, ts, nq, nt, nb, m2, o0, o1):
    ns = nt - nb
    c = x_hbm.shape[1]
    c4 = w1_hbm.shape[1]
    nk = c4 // L
    n3 = nk // 3
    nr = tm // ts
    tq = tm // nq
    m = ts // 2

    order0 = [int(ch, 16) for ch in o0]
    order1 = [int(ch, 16) for ch in o1]

    def rows(t, n=tm, off=0):
        return pl.ds(pl.multiple_of(t * tm + off, 128), n)

    def rot(j):
        if isinstance(j, int):
            return nt - 1 - j if j < nb else j - nb
        return jnp.where(j < nb, nt - 1 - j, j - nb)

    def xcopy(slot, t):
        return pltpu.make_async_copy(x_hbm.at[rows(t)], xbuf.at[slot], xsem.at[slot])

    def hcopy(slot, t):
        return pltpu.make_async_copy(x_hbm.at[rows(t, ts)], hbuf.at[slot], hsem.at[slot])

    def ocopy(slot, t, q):
        return pltpu.make_async_copy(xbuf.at[slot, pl.ds(q * tq, tq)], o_hbm.at[rows(t, tq, q * tq)],
                                     osem.at[slot])

    def owait(slot, t):
        for q in range(nq):
            ocopy(slot, t, q).wait()

    def wcopy(s, t):
        return pltpu.make_async_copy(ring.at[pl.ds(s * nq, nq)], h_hbm.at[pl.ds(t * nq, nq)], wsem.at[s])

    def rcopy(s, t, q):
        return pltpu.make_async_copy(h_hbm.at[t * nq + q], ring.at[s * nq + q], rsem.at[s * nq + q])

    def layernorm(xv):
        y = xv.astype(F32) * dw_ref[...].astype(F32)
        mu = jnp.sum(y, axis=-1, keepdims=True) * (1.0 / c)
        yc = y - mu
        var = jnp.mean(yc * yc, axis=-1, keepdims=True)
        xn = yc * (lax.rsqrt(var + 1e-5) * ALPHA)
        blocks = {i * 3 + j: xn[i * m:(i + 1) * m, j * L:(j + 1) * L] for i in range(2) for j in range(3)}
        return tuple(v.astype(BF16) for v in _eval_plan(_A_PLAN, blocks))

    def lhs_store(t):
        for q, v in enumerate(t):
            lhs0_ref[q] = v

    def act(z, slot, j, r0):
        t = jnp.tanh(z * (z * z + BETA))
        g = z * (t + 1.0)
        ssq_ref[:, j * L:(j + 1) * L] += jnp.sum((g * g).reshape(m // 8, 8, L), axis=0)
        rr = (j % n3) * tq + r0 % tq
        ring[slot * nq + r0 // tq, j // n3, rr:rr + m, :] = g.astype(BF16)

    def inc(v, n):
        return jnp.where(v + 1 >= n, 0, v + 1)

    def dec(v, n):
        return jnp.where(v == 0, n - 1, v - 1)

    last = nb * nq - 1
    cp_dw = pltpu.make_async_copy(dw_hbm, dw_ref, psem.at[0])
    cp_w1 = [pltpu.make_async_copy(w1_hbm.at[:, pl.ds(j * L, L)],
                                   ring.at[last, j // n3, pl.ds((j % n3) * tq, c)], psem.at[1])
             for j in range(nk)]
    cp_w2 = pltpu.make_async_copy(w2_hbm, xbuf.at[2, pl.ds(0, c4)], psem.at[2])
    cp_g = pltpu.make_async_copy(g_hbm, g_ref, psem.at[3])
    cp_b = pltpu.make_async_copy(b_hbm, b_ref, psem.at[4])
    cp_dw.start()
    hcopy(0, 0).start()
    for cp in cp_w1:
        cp.start()
    hcopy(1, 1).start()
    xcopy(0, 0).start(priority=1)
    cp_w2.start(priority=1)
    cp_g.start(priority=1)
    cp_b.start(priority=1)
    ssq_ref[...] = jnp.zeros(ssq_ref.shape, F32)
    for q in range(NP):
        zero_ref[q] = 0
    cp_dw.wait()
    hcopy(0, 0).wait()
    lhs_store(layernorm(hbuf[0]))
    for cp in cp_w1:
        cp.wait()
    for cc in range(n3):
        blocks = {j * 3 + l: ring[last, l, cc * tq + j * L:cc * tq + (j + 1) * L, :].astype(F32)
                  for j in range(3) for l in range(3)}
        for q, v in enumerate(_eval_plan(_B_PLAN, blocks)):
            wc_ref[q, cc * L // 2:(cc + 1) * L // 2, :] = _pack(v)

    def phase0(i, carry):
        xs, slot = carry
        xs1 = 1 - xs
        xcopy(xs, i).wait()
        hcopy(xs1, jnp.minimum(i + 1, nt - 1)).wait()

        @pl.when(i + 1 < nt)
        def _():
            xcopy(xs1, i + 1).start()
            hcopy(xs, jnp.minimum(i + 2, nt - 1)).start()

        @pl.when(i >= nb)
        def _():
            wcopy(slot, i - nb).wait()

        lhs = tuple(lhs0_ref[q] for q in range(NP))
        for k in range(nr):
            if k + 1 < nr:
                lhs_next = layernorm(xbuf[xs, (k + 1) * ts:(k + 2) * ts, :])
            else:
                lhs_next = layernorm(hbuf[xs1])
            for cc in range(n3):
                P = {}
                for r in order0:
                    P[r] = _mm(lhs[r], _unpack(wc_ref[r, cc * L // 2:(cc + 1) * L // 2, :]))
                for o, v in enumerate(_eval_plan(_C_PLAN, P)):
                    act(v, slot, (o % 3) * n3 + cc, k * ts + (o // 3) * m)
            lhs = lhs_next
        lhs_store(lhs)

        @pl.when(i < ns)
        def _():
            wcopy(slot, i).start(priority=1)

        return xs1, inc(slot, nb)

    lax.fori_loop(0, nt, phase0, (jnp.int32(0), jnp.int32(0)))

    cp_w2.wait()
    cp_g.wait()
    cp_b.wait()
    inv = 1.0 / (2.0 * ALPHA)
    ss = jnp.sum(ssq_ref[...], axis=0, keepdims=True) * (inv * inv)
    gx = jnp.sqrt(ss + 1e-6)
    nx = gx / (jnp.mean(gx, axis=-1, keepdims=True) + 1e-6)
    s = (g_ref[...].reshape(1, c4).astype(F32) * nx + 1.0) * inv
    k3 = c4 // 3
    for rb in range(k3 // L):
        blocks = {}
        for j in range(3):
            r0 = j * k3 + rb * L
            st = jnp.transpose(jnp.broadcast_to(s[:, r0:r0 + L], (L, L)))
            for l in range(3):
                blocks[j * 3 + l] = xbuf[2, r0:r0 + L, l * L:(l + 1) * L].astype(F32) * st
        for q, v in enumerate(_eval_plan(_B_PLAN, blocks)):
            wc_ref[q, rb * L // 2:(rb + 1) * L // 2, :] = _pack(v)
    bias_ref[...] = _mm(jnp.broadcast_to(b_ref[...].reshape(1, c4), (8, c4)), xbuf[2, 0:c4, :])

    def phase1(j, carry):
        xs, slot = carry
        xs1 = dec(xs, NX)

        @pl.when(j >= 2)
        def _():
            owait(xs1, rot(j - 2))

        @pl.when(jnp.logical_and(j >= 1, j + 1 < nt))
        def _():
            xcopy(xs1, rot(j + 1)).start()

        @pl.when(j >= 2)
        def _():
            xcopy(xs, rot(j)).wait()

        tile = rot(j)
        base = [slot * nq + zero_ref[r] for r in range(NP)]

        def A(r, row0, jk):
            q = row0 // tq
            cols = []
            for kt in range(n3):
                rr = kt * tq + row0 % tq
                cols.append(ring[base[r] + q, jk, rr:rr + m2, :])
            return jnp.concatenate(cols, axis=1)

        per_q = tq // (2 * m2)
        for k in range(tm // (2 * m2)):
            q = k // per_q
            if k % per_q == 0:
                @pl.when(j >= nb)
                def _():
                    rcopy(slot, j - nb, q).wait()
            r0 = (2 * k * m2, (2 * k + 1) * m2)
            P = {}
            for r in order1:
                terms = [(_U[r][i_][j_], (lambda i_=i_, j_=j_: A(r, r0[i_], j_)))
                         for i_ in range(2) for j_ in range(3) if _U[r][i_][j_]]
                if len(terms) == 1:
                    assert terms[0][0] == 1
                    lhs = terms[0][1]()
                else:
                    lhs = _signed_sum([(sg, (lambda t=t: t().astype(F32))) for sg, t in terms]).astype(BF16)
                P[r] = _mm(lhs, _unpack(wc_ref[r]))
            for o, v in enumerate(_eval_plan(_C_PLAN, P)):
                rs = slice(r0[o // 3], r0[o // 3] + m2)
                cs = slice((o % 3) * L, (o % 3 + 1) * L)
                xbuf[xs, rs, cs] = (v + xbuf[xs, rs, cs].astype(F32) + bias_ref[0:1, cs]).astype(BF16)
            if (k + 1) % per_q == 0:
                ocopy(xs, tile, q).start()

                @pl.when(j < ns)
                def _():
                    rcopy(slot, j, q).start(priority=1)

        return xs1, dec(slot, nb)

    lax.fori_loop(0, nt, phase1, (jnp.int32(1), jnp.int32((nt - 1) % nb)))
    owait((1 - (nt - 2)) % NX, rot(nt - 2))
    owait((1 - (nt - 1)) % NX, rot(nt - 1))


@jax.jit
def pallas_standalone__modern_conv_block_slak__vision_kernel(x, dw, w1, w2, grn_g, grn_b):
    tm, ts, nq, nb, m2 = 3072, 64, 3, 13, 128
    o0, o1 = '01b825ce97a64d3', '0123456789abcde'
    B, H, W, C = x.shape
    n = B * H * W
    c4 = w1.shape[1]
    nk = c4 // L
    nt = n // tm
    ns = nt - nb
    tq = tm // nq
    assert n % tm == 0 and nt % 2 == 0 and C == 3 * L and c4 == 12 * L and dw.shape[:2] == (1, 1)
    kern = functools.partial(_kernel, tm=tm, ts=ts, nq=nq, nt=nt, nb=nb, m2=m2, o0=o0, o1=o1)
    any_spec = pl.BlockSpec(memory_space=pl.ANY)
    out, _ = pl.pallas_call(
        kern,
        in_specs=[any_spec] * 6,
        out_specs=[any_spec, any_spec],
        out_shape=[jax.ShapeDtypeStruct((n, C), x.dtype),
                   jax.ShapeDtypeStruct((ns * nq, 3, nk // 3 * tq, L), BF16)],
        scratch_shapes=[
            pltpu.VMEM((NX, tm, C), BF16),
            pltpu.VMEM((2, ts, C), BF16),
            pltpu.VMEM((nb * nq, 3, nk // 3 * tq, L), BF16),
            pltpu.VMEM((8, c4), F32),
            pltpu.VMEM((1, C), BF16),
            pltpu.VMEM((c4,), BF16),
            pltpu.VMEM((c4,), BF16),
            pltpu.VMEM((NP, c4 // 6, L), U32),
            pltpu.VMEM((NP, ts // 2, L), BF16),
            pltpu.VMEM((8, C), F32),
            pltpu.SMEM((NP,), jnp.int32),
            pltpu.SemaphoreType.DMA((NX,)),
            pltpu.SemaphoreType.DMA((2,)),
            pltpu.SemaphoreType.DMA((NX,)),
            pltpu.SemaphoreType.DMA((nb,)),
            pltpu.SemaphoreType.DMA((nb * nq,)),
            pltpu.SemaphoreType.DMA((5,)),
        ],
        compiler_params=pltpu.CompilerParams(
            disable_bounds_checks=True,
            vmem_limit_bytes=128 * 1024 * 1024),
    )(x.reshape(n, C), dw.reshape(1, C), w1, w2, grn_g, grn_b)
    return out.reshape(B, H, W, C)
```
